```python
import jax
import jax.numpy as jnp

def _softmax(x, axis=-1):
    return jax.nn.softmax(x, axis=axis)
def _gelu(x):
    return jax.nn.gelu(x, approximate=True)
def _silu(x):
    return jax.nn.silu(x)
def _sigmoid(x):
    return jax.nn.sigmoid(x)
def _layernorm(x, axis=-1, eps=1e-5):
    m = jnp.mean(x, axis=axis, keepdims=True)
    v = jnp.var(x, axis=axis, keepdims=True)
    return (x - m) / jnp.sqrt(v + eps)
def _scatter_add(tgt, idx, src, axis=0):
    return tgt.at[idx].add(src)
def _segment_sum(src, seg, n):
    return jax.ops.segment_sum(src, seg, n)
class _Rng:
    def __init__(self, key):
        self._k = key
    def _next(self):
        self._k, sub = jax.random.split(self._k)
        return sub
    def normal(self, shape):
        return jax.random.normal(self._next(), shape, dtype=jnp.bfloat16)
    def randint(self, lo, hi, shape):
        return jax.random.randint(self._next(), shape, lo, hi, dtype=jnp.int32)
    def uniform(self, shape, lo=0.0, hi=1.0):
        return jax.random.uniform(self._next(), shape, jnp.bfloat16, lo, hi)
    def permutation(self, n):
        return jax.random.permutation(self._next(), n)


kernel_name = 'standalone__cross_network_dcn_v2__recsys'

def setup_inputs():
    _rng = _Rng(jax.random.key(int.from_bytes(__import__("os").urandom(4), "little")))
    _w = (lambda a: (lambda t: t.astype(jnp.bfloat16) if jnp.issubdtype(t.dtype, jnp.floating) else t)(jnp.asarray(a)))
    B, F, D, L = 16384, 100, 16, 3
    Din = min(F * D, 512)
    R = max(Din // 4, 2)
    sc = Din ** -0.5
    return {
        "x0": _w((lambda *s: _rng.normal(s) * 0.05)(B, Din)),
        "U":  _w((lambda *s: _rng.normal(s) * 0.05)(L, Din, R) * sc),
        "V":  _w((lambda *s: _rng.normal(s) * 0.05)(L, R, Din) * sc),
        "bs": _w((lambda *s: _rng.normal(s) * 0.05)(L, Din)),
    }

def reference(x0, U, V, bs):
    x = x0
    for l in range(U.shape[0]):
        h = jnp.einsum('rd,bd->br', V[l], x)
        h = jnp.einsum('dr,br->bd', U[l], h)
        x = x0 * (h + bs[l]) + x
    return x
```

```python
import jax
import jax.numpy as jnp
import jax.experimental.pallas as pl
import jax.experimental.pallas.tpu as pltpu

_NT = (((1,), (1,)), ((), ()))

_HEAD = (256, 640, 1952)
_BODY = (1024, 1024, 1024, 768, 416, 256)
_STEPS = 3
_PIECE = 128


def _kernel(x_hbm, u_hbm, v_hbm, b_hbm, o_hbm,
            x_v, o_v, u_v, v_v, b_v, in_sems, w_sems, out_sem):
    f32, bf16 = jnp.float32, jnp.bfloat16
    n_layers = u_hbm.shape[0]
    n_head = len(_HEAD)
    head_start = [sum(_HEAD[:i]) for i in range(n_head + 1)]
    step_rows = sum(_BODY)

    def in_copy(start, size, i):
        r = pl.ds(start, size)
        return pltpu.make_async_copy(x_hbm.at[r], x_v.at[r], in_sems.at[i])

    def out_copy(start, size):
        r = pl.ds(start, size)
        return pltpu.make_async_copy(o_v.at[r], o_hbm.at[r], out_sem.at[0])

    weight_copies = [
        pltpu.make_async_copy(v_hbm, v_v, w_sems.at[0]),
        pltpu.make_async_copy(u_hbm, u_v, w_sems.at[1]),
        pltpu.make_async_copy(b_hbm, b_v, w_sems.at[2]),
    ]

    def cross(start, size, piece):
        x0 = x_v[pl.ds(start, size), :]
        x = x0
        for l in range(n_layers):
            h = jax.lax.dot_general(x, v_v[l], _NT, preferred_element_type=f32)
            h = jax.lax.dot_general(h.astype(bf16), u_v[l], _NT,
                                    preferred_element_type=f32)
            b = b_v[pl.ds(l, 1), :].astype(f32)
            if l == 0:
                x = (x0.astype(f32) * (h + (b + 1.0))).astype(bf16)
            else:
                x = (x0.astype(f32) * (h + b) + x.astype(f32)).astype(bf16)
        for s in range(0, size, piece):
            m = min(piece, size - s)
            st = start + s
            if not isinstance(st, int):
                st = pl.multiple_of(st, 16)
            o_v[pl.ds(st, m), :] = x[s:s + m]
            out_copy(st, m).start(priority=1)

    in_copy(0, _HEAD[0], 0).start()
    for c in weight_copies:
        c.start()
    for i in range(1, n_head):
        in_copy(head_start[i], _HEAD[i], i).start(priority=1)
    for i in range(_STEPS):
        in_copy(head_start[-1] + i * step_rows, step_rows, n_head + i).start(priority=1)

    for c in weight_copies:
        c.wait()
    for i in range(n_head):
        in_copy(head_start[i], _HEAD[i], i).wait()
        cross(head_start[i], _HEAD[i], _HEAD[i])

    def step(i, carry):
        base = pl.multiple_of(head_start[-1] + i * step_rows, 16)
        in_copy(base, step_rows, n_head + i).wait()
        s = 0
        for j, m in enumerate(_BODY):
            cross(pl.multiple_of(base + s, 16), m,
                  _PIECE if j >= len(_BODY) - 2 else m)
            s += m
        return carry

    jax.lax.fori_loop(0, _STEPS, step, 0)
    pltpu.make_async_copy(o_v, o_hbm, out_sem.at[0]).wait()


@jax.jit
def pallas_standalone__cross_network_dcn_v2__recsys_kernel(
    x0: jax.Array,
    U: jax.Array,
    V: jax.Array,
    bs: jax.Array,
):
    B, D = x0.shape
    assert B == sum(_HEAD) + _STEPS * sum(_BODY)
    any_spec = pl.BlockSpec(memory_space=pl.ANY)
    return pl.pallas_call(
        _kernel,
        in_specs=[any_spec] * 4,
        out_specs=any_spec,
        out_shape=jax.ShapeDtypeStruct((B, D), x0.dtype),
        scratch_shapes=[
            pltpu.VMEM((B, D), x0.dtype),
            pltpu.VMEM((B, D), x0.dtype),
            pltpu.VMEM(U.shape, U.dtype),
            pltpu.VMEM(V.shape, V.dtype),
            pltpu.VMEM(bs.shape, bs.dtype),
            pltpu.SemaphoreType.DMA((len(_HEAD) + _STEPS,)),
            pltpu.SemaphoreType.DMA((3,)),
            pltpu.SemaphoreType.DMA((1,)),
        ],
        compiler_params=pltpu.CompilerParams(vmem_limit_bytes=100 * 1024 * 1024),
    )(x0, U, V, bs)
```

```python
import jax
import jax.numpy as jnp
import jax.experimental.pallas as pl
import jax.experimental.pallas.tpu as pltpu

_NT = (((1,), (1,)), ((), ()))

_STEPS = 2
_CHUNKS = (320, 224, 688, 880, 864, 1024, 1024, 1024, 1024, 608, 320, 192)
_IN_GROUPS = (0, 1, 2, 3, 5, 10, len(_CHUNKS))
_SHIP_FROM = 6
_OUT_PIECES = {10: (128, 128, 64), 11: (32, 32, 64, 64)}

_OFFSETS = tuple(sum(_CHUNKS[:c]) for c in range(len(_CHUNKS) + 1))
_STEP_ROWS = _OFFSETS[-1]
_N_GROUPS = len(_IN_GROUPS) - 1


def _kernel(x_hbm, u_hbm, v_hbm, b_hbm, o_hbm, x_v, o_v, u_v, v_v, b_v, sems):
    f32, bf16 = jnp.float32, jnp.bfloat16
    n_layers = u_hbm.shape[0]
    n_matmuls = 2 * n_layers
    sem_rest = _N_GROUPS + n_matmuls - 2
    sem_out = sem_rest + 1

    def x_copy(lo, hi, sem):
        rows = pl.ds(lo, hi - lo)
        return pltpu.make_async_copy(x_hbm.at[rows], x_v.at[rows], sems.at[sem])

    def out_copy(start, size):
        rows = pl.ds(start, size)
        return pltpu.make_async_copy(o_v.at[rows], o_hbm.at[rows], sems.at[sem_out])

    def weight_copy(k, sem):
        src, dst = (v_hbm, v_v) if k % 2 == 0 else (u_hbm, u_v)
        return pltpu.make_async_copy(src.at[k // 2], dst.at[k // 2], sems.at[sem])

    group_copies = {
        _IN_GROUPS[g]: x_copy(_OFFSETS[_IN_GROUPS[g]], _OFFSETS[_IN_GROUPS[g + 1]], g)
        for g in range(1, _N_GROUPS)
    }
    first_copies = [
        weight_copy(0, 0),
        x_copy(0, _OFFSETS[_IN_GROUPS[1]], 0),
        weight_copy(1, 0),
        pltpu.make_async_copy(b_hbm, b_v, sems.at[0]),
    ]
    weight_copies = {k: weight_copy(k, _N_GROUPS + k - 2) for k in range(2, n_matmuls)}
    rest_copy = x_copy(_STEP_ROWS, _STEPS * _STEP_ROWS, sem_rest)

    for copy in first_copies + list(weight_copies.values()):
        copy.start()
    for copy in list(group_copies.values()) + [rest_copy]:
        copy.start(priority=1)

    def wait_if(cond, copies):
        @pl.when(cond)
        def _():
            for copy in copies:
                copy.wait()

    def step(i, carry):
        first = i == 0
        base = i * _STEP_ROWS
        wait_if(i == 1, [rest_copy])
        wait_if(first, first_copies)
        for c, size in enumerate(_CHUNKS):
            start = pl.multiple_of(base + _OFFSETS[c], 16)
            x0 = x_v[pl.ds(start, size), :]
            x = x0
            for l in range(n_layers):
                if c == 0 and l > 0:
                    wait_if(first, [weight_copies[2 * l]])
                h = jax.lax.dot_general(x, v_v[l], _NT, preferred_element_type=f32)
                if c == 0 and l > 0:
                    wait_if(first, [weight_copies[2 * l + 1]])
                u = u_v[l]
                if l == n_layers - 1 and c + 1 in group_copies:
                    wait_if(first, [group_copies[c + 1]])
                h = jax.lax.dot_general(h.astype(bf16), u, _NT,
                                        preferred_element_type=f32)
                b = b_v[pl.ds(l, 1), :].astype(f32)
                if l == 0:
                    x = (x0.astype(f32) * (h + (b + 1.0))).astype(bf16)
                else:
                    x = (x0.astype(f32) * (h + b) + x.astype(f32)).astype(bf16)

            done = 0
            for rows in _OUT_PIECES.get(c, (size,)):
                piece = pl.multiple_of(start + done, 16)
                o_v[pl.ds(piece, rows), :] = x[done:done + rows]
                if c >= _SHIP_FROM:
                    out_copy(piece, rows).start(priority=1)
                done += rows
            if c == _SHIP_FROM - 1:
                out_copy(pl.multiple_of(base, 16), _OFFSETS[c + 1]).start(priority=1)
        return carry

    jax.lax.fori_loop(0, _STEPS, step, 0)
    pltpu.make_async_copy(o_v, o_hbm, sems.at[sem_out]).wait()


@jax.jit
def pallas_standalone__cross_network_dcn_v2__recsys_kernel(
    x0: jax.Array,
    U: jax.Array,
    V: jax.Array,
    bs: jax.Array,
):
    B, D = x0.shape
    assert B == _STEPS * _STEP_ROWS
    in_hbm = pl.BlockSpec(memory_space=pl.ANY)
    return pl.pallas_call(
        _kernel,
        in_specs=[in_hbm] * 4,
        out_specs=in_hbm,
        out_shape=jax.ShapeDtypeStruct((B, D), x0.dtype),
        scratch_shapes=[
            pltpu.VMEM((B, D), x0.dtype),
            pltpu.VMEM((B, D), x0.dtype),
            pltpu.VMEM(U.shape, U.dtype),
            pltpu.VMEM(V.shape, V.dtype),
            pltpu.VMEM(bs.shape, bs.dtype),
            pltpu.SemaphoreType.DMA((_N_GROUPS + 2 * U.shape[0],)),
        ],
        compiler_params=pltpu.CompilerParams(
            vmem_limit_bytes=100 * 1024 * 1024,
            flags={"XLA_TPU_RESCHEDULE_DMA_DONES": True},
        ),
    )(x0, U, V, bs)
```

```python
import jax
import jax.numpy as jnp
import jax.experimental.pallas as pl
import jax.experimental.pallas.tpu as pltpu

_NT = (((1,), (1,)), ((), ()))
_TILE = 16

_STEPS = 2
_CHUNKS = (288, 192, 480, 1024, 1024, 1024, 1024, 1024, 1024, 576, 320, 192)
_IN_GROUPS = (0, 1, 2, 3, 4, 7, len(_CHUNKS))
_SHIP_FROM = 6
_OUT_PIECES = {10: (128, 128, 64), 11: (32, 32, 64, 64)}

_WEIGHT_WAIT_ROW = {1: 48, 2: 96, 3: 48, 4: 48, 5: 48}
_X_WAIT_AFTER_ROWS = {1: 64, 3: 256}
_X_WAIT_V_ROW = {2: 112}

_OFFSETS = tuple(sum(_CHUNKS[:c]) for c in range(len(_CHUNKS) + 1))
_STEP_ROWS = _OFFSETS[-1]
_N_GROUPS = len(_IN_GROUPS) - 1


def _kernel(x_hbm, u_hbm, v_hbm, b_hbm, o_hbm, x_v, o_v, u_v, v_v, b_v, sems):
    f32, bf16 = jnp.float32, jnp.bfloat16
    n_layers = u_hbm.shape[0]
    n_matmuls = 2 * n_layers
    sem_rest = _N_GROUPS + n_matmuls - 1
    sem_out = sem_rest + 1

    def x_copy(lo, hi, sem):
        rows = pl.ds(lo, hi - lo)
        return pltpu.make_async_copy(x_hbm.at[rows], x_v.at[rows], sems.at[sem])

    def out_copy(start, size):
        rows = pl.ds(start, size)
        return pltpu.make_async_copy(o_v.at[rows], o_hbm.at[rows], sems.at[sem_out])

    def weight_copy(k, sem):
        src, dst = (v_hbm, v_v) if k % 2 == 0 else (u_hbm, u_v)
        return pltpu.make_async_copy(src.at[k // 2], dst.at[k // 2], sems.at[sem])

    first_copies = [weight_copy(0, 0), x_copy(0, _OFFSETS[_IN_GROUPS[1]], 0)]
    weight_copies = {
        k: [weight_copy(k, _N_GROUPS + k - 1)] for k in range(1, n_matmuls)
    }
    weight_copies[1].append(pltpu.make_async_copy(b_hbm, b_v, sems.at[_N_GROUPS]))
    group_copies = {
        _IN_GROUPS[g]: x_copy(_OFFSETS[_IN_GROUPS[g]], _OFFSETS[_IN_GROUPS[g + 1]], g)
        for g in range(1, _N_GROUPS)
    }
    rest_copy = x_copy(_STEP_ROWS, _STEPS * _STEP_ROWS, sem_rest)

    for copy in first_copies:
        copy.start()
    for k in range(1, n_matmuls):
        for copy in weight_copies[k]:
            copy.start()
    for copy in list(group_copies.values()) + [rest_copy]:
        copy.start(priority=1)

    def wait_if(cond, copies):
        @pl.when(cond)
        def _():
            for copy in copies:
                copy.wait()

    def step(i, carry):
        first = i == 0
        base = i * _STEP_ROWS
        wait_if(i == 1, [rest_copy])
        wait_if(first, first_copies)
        v_next = None
        for c, size in enumerate(_CHUNKS):
            start = pl.multiple_of(base + _OFFSETS[c], _TILE)

            def store_early(value, row):
                rows = pl.ds(pl.multiple_of(start + row, _TILE), _TILE)
                o_v[rows, pl.ds(0, value.shape[1])] = value[row:row + _TILE]

            x0 = x_v[pl.ds(start, size), :]
            x = x0
            for l in range(n_layers):
                if c == 0 and l > 0:
                    store_early(x, _WEIGHT_WAIT_ROW[2 * l])
                    wait_if(first, weight_copies[2 * l])
                v = v_v[l] if v_next is None else v_next
                v_next = None
                h = jax.lax.dot_general(x, v, _NT, preferred_element_type=f32)
                h = h.astype(bf16)
                if c == 0:
                    store_early(h, _WEIGHT_WAIT_ROW[2 * l + 1])
                    wait_if(first, weight_copies[2 * l + 1])
                u = u_v[l]
                if (l == n_layers - 1 and c + 1 in group_copies
                        and c + 1 not in _X_WAIT_AFTER_ROWS):
                    if c + 1 in _X_WAIT_V_ROW:
                        store_early(h, _X_WAIT_V_ROW[c + 1])
                    wait_if(first, [group_copies[c + 1]])
                h = jax.lax.dot_general(h, u, _NT, preferred_element_type=f32)
                b = b_v[pl.ds(l, 1), :].astype(f32)
                if l == 0:
                    x = (x0.astype(f32) * (h + (b + 1.0))).astype(bf16)
                else:
                    x = (x0.astype(f32) * (h + b) + x.astype(f32)).astype(bf16)

            pieces = _OUT_PIECES.get(c, (size,))
            if c + 1 in _X_WAIT_AFTER_ROWS:
                pieces = (_X_WAIT_AFTER_ROWS[c + 1], size - _X_WAIT_AFTER_ROWS[c + 1])
            done = 0
            for rows in pieces:
                piece = pl.multiple_of(start + done, _TILE)
                o_v[pl.ds(piece, rows), :] = x[done:done + rows]
                if c >= _SHIP_FROM:
                    out_copy(piece, rows).start(priority=1)
                if done == 0 and c + 1 in _X_WAIT_AFTER_ROWS:
                    v_next = v_v[0]
                    wait_if(first, [group_copies[c + 1]])
                done += rows
            if c == _SHIP_FROM - 1:
                out_copy(pl.multiple_of(base, _TILE), _OFFSETS[c + 1]).start(priority=1)
        return carry

    jax.lax.fori_loop(0, _STEPS, step, 0)
    pltpu.make_async_copy(o_v, o_hbm, sems.at[sem_out]).wait()


@jax.jit
def pallas_standalone__cross_network_dcn_v2__recsys_kernel(
    x0: jax.Array,
    U: jax.Array,
    V: jax.Array,
    bs: jax.Array,
):
    B, D = x0.shape
    assert B == _STEPS * _STEP_ROWS and U.shape[0] == 3
    in_hbm = pl.BlockSpec(memory_space=pl.ANY)
    return pl.pallas_call(
        _kernel,
        in_specs=[in_hbm] * 4,
        out_specs=in_hbm,
        out_shape=jax.ShapeDtypeStruct((B, D), x0.dtype),
        scratch_shapes=[
            pltpu.VMEM((B, D), x0.dtype),
            pltpu.VMEM((B, D), x0.dtype),
            pltpu.VMEM(U.shape, U.dtype),
            pltpu.VMEM(V.shape, V.dtype),
            pltpu.VMEM(bs.shape, bs.dtype),
            pltpu.SemaphoreType.DMA((_N_GROUPS + 2 * U.shape[0] + 1,)),
        ],
        compiler_params=pltpu.CompilerParams(
            vmem_limit_bytes=100 * 1024 * 1024,
            flags={"XLA_TPU_RESCHEDULE_DMA_DONES": True},
        ),
    )(x0, U, V, bs)
```

```python
import functools

import jax
import jax.numpy as jnp
import jax.experimental.pallas as pl
import jax.experimental.pallas.tpu as pltpu

_NT = (((1,), (1,)), ((), ()))
_TILE = 16

_STEPS = 2
_CHUNKS = (288, 192, 480, 1024, 1024, 1024, 1024, 1024, 1024, 576, 320, 192)
_IN_GROUPS = (0, 1, 2, 3, 4, 7, len(_CHUNKS))
_SHIP_FROM = 6
_OUT_PIECES = {10: (128, 128, 64), 11: (32, 32, 64, 64)}

_WEIGHT_WAIT_ROW = {1: 48, 2: 96, 3: 48, 4: 48, 5: 48}
_X_WAIT_AFTER_ROWS = {1: 64, 3: 256}
_X_WAIT_V_ROW = {2: 112}

_OFFSETS = tuple(sum(_CHUNKS[:c]) for c in range(len(_CHUNKS) + 1))
_STEP_ROWS = _OFFSETS[-1]
_N_GROUPS = len(_IN_GROUPS) - 1


def _cross_network(x_hbm, u_hbm, v_hbm, b_hbm, o_hbm, x_v, o_v, u_v, v_v, b_v, sems):
    f32, bf16 = jnp.float32, jnp.bfloat16
    n_layers = u_hbm.shape[0]
    n_matmuls = 2 * n_layers
    sem_rest = _N_GROUPS + n_matmuls - 1
    sem_out = sem_rest + 1

    def x_copy(lo, hi, sem):
        rows = pl.ds(lo, hi - lo)
        return pltpu.make_async_copy(x_hbm.at[rows], x_v.at[rows], sems.at[sem])

    def out_copy(start, size):
        rows = pl.ds(start, size)
        return pltpu.make_async_copy(o_v.at[rows], o_hbm.at[rows], sems.at[sem_out])

    def weight_copy(k, sem):
        src, dst = (v_hbm, v_v) if k % 2 == 0 else (u_hbm, u_v)
        return pltpu.make_async_copy(src.at[k // 2], dst.at[k // 2], sems.at[sem])

    first_copies = [weight_copy(0, 0), x_copy(0, _OFFSETS[_IN_GROUPS[1]], 0)]
    weight_copies = {
        k: [weight_copy(k, _N_GROUPS + k - 1)] for k in range(1, n_matmuls)
    }
    weight_copies[1].append(pltpu.make_async_copy(b_hbm, b_v, sems.at[_N_GROUPS]))
    group_copies = {
        _IN_GROUPS[g]: x_copy(_OFFSETS[_IN_GROUPS[g]], _OFFSETS[_IN_GROUPS[g + 1]], g)
        for g in range(1, _N_GROUPS)
    }
    rest_copy = x_copy(_STEP_ROWS, _STEPS * _STEP_ROWS, sem_rest)

    for copy in first_copies:
        copy.start()
    for k in range(1, n_matmuls):
        for copy in weight_copies[k]:
            copy.start()
    for copy in list(group_copies.values()) + [rest_copy]:
        copy.start(priority=1)

    def wait_if(cond, copies):
        @pl.when(cond)
        def _():
            for copy in copies:
                copy.wait()

    def step(i, carry):
        first = i == 0
        base = i * _STEP_ROWS
        wait_if(i == 1, [rest_copy])
        wait_if(first, first_copies)
        v_next = None
        for c, size in enumerate(_CHUNKS):
            start = pl.multiple_of(base + _OFFSETS[c], _TILE)

            def store_early(value, row):
                rows = pl.ds(pl.multiple_of(start + row, _TILE), _TILE)
                o_v[rows, pl.ds(0, value.shape[1])] = value[row:row + _TILE]

            x0 = x_v[pl.ds(start, size), :]
            x = x0
            for l in range(n_layers):
                if c == 0 and l > 0:
                    store_early(x, _WEIGHT_WAIT_ROW[2 * l])
                    wait_if(first, weight_copies[2 * l])
                v = v_v[l] if v_next is None else v_next
                v_next = None
                h = jax.lax.dot_general(x, v, _NT, preferred_element_type=f32)
                h = h.astype(bf16)
                if c == 0:
                    store_early(h, _WEIGHT_WAIT_ROW[2 * l + 1])
                    wait_if(first, weight_copies[2 * l + 1])
                u = u_v[l]
                if (l == n_layers - 1 and c + 1 in group_copies
                        and c + 1 not in _X_WAIT_AFTER_ROWS):
                    if c + 1 in _X_WAIT_V_ROW:
                        store_early(h, _X_WAIT_V_ROW[c + 1])
                    wait_if(first, [group_copies[c + 1]])
                h = jax.lax.dot_general(h, u, _NT, preferred_element_type=f32)
                b = b_v[pl.ds(l, 1), :].astype(f32)
                if l == 0:
                    x = (x0.astype(f32) * (h + (b + 1.0))).astype(bf16)
                else:
                    x = (x0.astype(f32) * (h + b) + x.astype(f32)).astype(bf16)

            pieces = _OUT_PIECES.get(c, (size,))
            if c + 1 in _X_WAIT_AFTER_ROWS:
                pieces = (_X_WAIT_AFTER_ROWS[c + 1], size - _X_WAIT_AFTER_ROWS[c + 1])
            done = 0
            for rows in pieces:
                piece = pl.multiple_of(start + done, _TILE)
                o_v[pl.ds(piece, rows), :] = x[done:done + rows]
                if c >= _SHIP_FROM:
                    out_copy(piece, rows).start(priority=1)
                if done == 0 and c + 1 in _X_WAIT_AFTER_ROWS:
                    v_next = v_v[0]
                    wait_if(first, [group_copies[c + 1]])
                done += rows
            if c == _SHIP_FROM - 1:
                out_copy(pl.multiple_of(base, _TILE), _OFFSETS[c + 1]).start(priority=1)
        return carry

    jax.lax.fori_loop(0, _STEPS, step, 0)
    pltpu.make_async_copy(o_v, o_hbm, sems.at[sem_out]).wait()


def _kernel(x_hbm, u_hbm, *refs):
    pl.run_scoped(
        functools.partial(_cross_network, x_hbm, u_hbm, *refs),
        pltpu.SemaphoreType.DMA((_N_GROUPS + 2 * u_hbm.shape[0] + 1,)),
    )


@jax.jit
def pallas_standalone__cross_network_dcn_v2__recsys_kernel(
    x0: jax.Array,
    U: jax.Array,
    V: jax.Array,
    bs: jax.Array,
):
    B, D = x0.shape
    assert B == _STEPS * _STEP_ROWS and U.shape[0] == 3
    in_hbm = pl.BlockSpec(memory_space=pl.ANY)
    return pl.pallas_call(
        _kernel,
        in_specs=[in_hbm] * 4,
        out_specs=in_hbm,
        out_shape=jax.ShapeDtypeStruct((B, D), x0.dtype),
        scratch_shapes=[
            pltpu.VMEM((B, D), x0.dtype),
            pltpu.VMEM((B, D), x0.dtype),
            pltpu.VMEM(U.shape, U.dtype),
            pltpu.VMEM(V.shape, V.dtype),
            pltpu.VMEM(bs.shape, bs.dtype),
        ],
        compiler_params=pltpu.CompilerParams(
            vmem_limit_bytes=100 * 1024 * 1024,
            flags={"XLA_TPU_RESCHEDULE_DMA_DONES": True},
        ),
    )(x0, U, V, bs)
```

```python
import functools

import jax
import jax.numpy as jnp
import jax.experimental.pallas as pl
import jax.experimental.pallas.tpu as pltpu

_NT = (((1,), (1,)), ((), ()))
_TILE = 16

_STEPS = 2
_CHUNKS = (288, 192, 480, 1024, 1024, 1024, 1024, 1024, 1024, 576, 320, 192)
_IN_GROUPS = (0, 1, 2, 3, 4, 7, len(_CHUNKS))
_SHIP_FROM = 6
_OUT_PIECES = {10: (128, 128, 64), 11: (32, 32, 64, 64)}

_WEIGHT_WAIT_ROW = 48
_X_WAIT_AFTER_ROWS = {1: 48, 3: 256}
_X_WAIT_V_ROW = {2: 112}

_OFFSETS = tuple(sum(_CHUNKS[:c]) for c in range(len(_CHUNKS) + 1))
_STEP_ROWS = _OFFSETS[-1]
_N_GROUPS = len(_IN_GROUPS) - 1


def _cross_network(x_hbm, u_hbm, v_hbm, b_hbm, o_hbm, x_v, o_v, u_v, v_v, b_v, sems):
    f32, bf16 = jnp.float32, jnp.bfloat16
    n_layers = u_hbm.shape[0]
    n_matmuls = 2 * n_layers
    sem_rest = _N_GROUPS + n_matmuls - 1
    sem_out = sem_rest + 1

    def x_copy(lo, hi, sem):
        rows = pl.ds(lo, hi - lo)
        return pltpu.make_async_copy(x_hbm.at[rows], x_v.at[rows], sems.at[sem])

    def out_copy(start, size):
        rows = pl.ds(start, size)
        return pltpu.make_async_copy(o_v.at[rows], o_hbm.at[rows], sems.at[sem_out])

    def weight_copy(k, sem):
        src, dst = (v_hbm, v_v) if k % 2 == 0 else (u_hbm, u_v)
        return pltpu.make_async_copy(src.at[k // 2], dst.at[k // 2], sems.at[sem])

    first_copies = [weight_copy(0, 0), x_copy(0, _OFFSETS[_IN_GROUPS[1]], 0)]
    weight_copies = {
        k: [weight_copy(k, _N_GROUPS + k - 1)] for k in range(1, n_matmuls)
    }
    weight_copies[1].append(pltpu.make_async_copy(b_hbm, b_v, sems.at[_N_GROUPS]))
    group_copies = {
        _IN_GROUPS[g]: x_copy(_OFFSETS[_IN_GROUPS[g]], _OFFSETS[_IN_GROUPS[g + 1]], g)
        for g in range(1, _N_GROUPS)
    }
    rest_copy = x_copy(_STEP_ROWS, _STEPS * _STEP_ROWS, sem_rest)

    for copy in first_copies:
        copy.start()
    for k in range(1, n_matmuls):
        for copy in weight_copies[k]:
            copy.start()
    for copy in list(group_copies.values()) + [rest_copy]:
        copy.start(priority=1)

    def wait_if(cond, copies):
        @pl.when(cond)
        def _():
            for copy in copies:
                copy.wait()

    def step(i, carry):
        first = i == 0
        base = i * _STEP_ROWS
        wait_if(i == 1, [rest_copy])
        wait_if(first, first_copies)
        v_next = None
        for c, size in enumerate(_CHUNKS):
            start = pl.multiple_of(base + _OFFSETS[c], _TILE)

            def store_early(value, row):
                rows = pl.ds(pl.multiple_of(start + row, _TILE), _TILE)
                o_v[rows, pl.ds(0, value.shape[1])] = value[row:row + _TILE]

            x0 = x_v[pl.ds(start, size), :]
            x = x0
            for l in range(n_layers):
                if c == 0 and l > 0:
                    store_early(x, _WEIGHT_WAIT_ROW)
                    wait_if(first, weight_copies[2 * l])
                v = v_v[l] if v_next is None else v_next
                v_next = None
                h = jax.lax.dot_general(x, v, _NT, preferred_element_type=f32)
                h = h.astype(bf16)
                if c == 0:
                    store_early(h, _WEIGHT_WAIT_ROW)
                    wait_if(first, weight_copies[2 * l + 1])
                u = u_v[l]
                if (l == n_layers - 1 and c + 1 in group_copies
                        and c + 1 not in _X_WAIT_AFTER_ROWS):
                    if c + 1 in _X_WAIT_V_ROW:
                        store_early(h, _X_WAIT_V_ROW[c + 1])
                    wait_if(first, [group_copies[c + 1]])
                h = jax.lax.dot_general(h, u, _NT, preferred_element_type=f32)
                b = b_v[pl.ds(l, 1), :].astype(f32)
                if l == 0:
                    x = (x0.astype(f32) * (h + (b + 1.0))).astype(bf16)
                else:
                    x = (x0.astype(f32) * (h + b) + x.astype(f32)).astype(bf16)

            pieces = _OUT_PIECES.get(c, (size,))
            if c + 1 in _X_WAIT_AFTER_ROWS:
                pieces = (_X_WAIT_AFTER_ROWS[c + 1], size - _X_WAIT_AFTER_ROWS[c + 1])
            done = 0
            for rows in pieces:
                piece = pl.multiple_of(start + done, _TILE)
                o_v[pl.ds(piece, rows), :] = x[done:done + rows]
                if c >= _SHIP_FROM:
                    out_copy(piece, rows).start(priority=1)
                if done == 0 and c + 1 in _X_WAIT_AFTER_ROWS:
                    v_next = v_v[0]
                    wait_if(first, [group_copies[c + 1]])
                done += rows
            if c == _SHIP_FROM - 1:
                out_copy(pl.multiple_of(base, _TILE), _OFFSETS[c + 1]).start(priority=1)
        return carry

    jax.lax.fori_loop(0, _STEPS, step, 0)
    pltpu.make_async_copy(o_v, o_hbm, sems.at[sem_out]).wait()


def _kernel(x_hbm, u_hbm, *refs):
    pl.run_scoped(
        functools.partial(_cross_network, x_hbm, u_hbm, *refs),
        pltpu.SemaphoreType.DMA((_N_GROUPS + 2 * u_hbm.shape[0] + 1,)),
    )


@jax.jit
def pallas_standalone__cross_network_dcn_v2__recsys_kernel(
    x0: jax.Array,
    U: jax.Array,
    V: jax.Array,
    bs: jax.Array,
):
    B, D = x0.shape
    assert B == _STEPS * _STEP_ROWS
    in_hbm = pl.BlockSpec(memory_space=pl.ANY)
    return pl.pallas_call(
        _kernel,
        in_specs=[in_hbm] * 4,
        out_specs=in_hbm,
        out_shape=jax.ShapeDtypeStruct((B, D), x0.dtype),
        scratch_shapes=[
            pltpu.VMEM((B, D), x0.dtype),
            pltpu.VMEM((B, D), x0.dtype),
            pltpu.VMEM(U.shape, U.dtype),
            pltpu.VMEM(V.shape, V.dtype),
            pltpu.VMEM(bs.shape, bs.dtype),
        ],
        compiler_params=pltpu.CompilerParams(
            vmem_limit_bytes=100 * 1024 * 1024,
            flags={"XLA_TPU_RESCHEDULE_DMA_DONES": True},
        ),
    )(x0, U, V, bs)
```
